```python
import os as _os
_os.environ.setdefault("JAX_PLATFORMS", "cpu")
import jax
import jax.numpy as jnp

def _softmax(x, axis=-1):
    return jax.nn.softmax(x, axis=axis)
def _gelu(x):
    return jax.nn.gelu(x, approximate=True)
def _silu(x):
    return jax.nn.silu(x)
def _sigmoid(x):
    return jax.nn.sigmoid(x)
def _layernorm(x, axis=-1, eps=1e-5):
    m = jnp.mean(x, axis=axis, keepdims=True)
    v = jnp.var(x, axis=axis, keepdims=True)
    return (x - m) / jnp.sqrt(v + eps)
def _scatter_add(tgt, idx, src, axis=0):
    return tgt.at[idx].add(src)
def _segment_sum(src, seg, n):
    return jax.ops.segment_sum(src, seg, n)
class _Rng:
    def __init__(self, key):
        self._k = key
    def _next(self):
        self._k, sub = jax.random.split(self._k)
        return sub
    def normal(self, shape):
        return jax.random.normal(self._next(), shape, dtype=jnp.bfloat16)
    def randint(self, lo, hi, shape):
        return jax.random.randint(self._next(), shape, lo, hi, dtype=jnp.int32)
    def uniform(self, shape, lo=0.0, hi=1.0):
        return jax.random.uniform(self._next(), shape, jnp.bfloat16, lo, hi)
    def permutation(self, n):
        return jax.random.permutation(self._next(), n)


kernel_name = 'sequential_preLN__linear_kernel_hedgehog__dense_activation_squared_relu__prompt'

def setup_inputs():
    _rng = _Rng(jax.random.key(int.from_bytes(__import__("os").urandom(4), "little")))
    _w = (lambda a: (lambda t: t.astype(jnp.bfloat16) if jnp.issubdtype(t.dtype, jnp.floating) else t)(jnp.asarray(a)))
    def _A_setup():
        B, S, D, H = 1, 2048, 512, 32
        Dh = D // H
        return {
            "x": _w((lambda *s: _rng.normal(s) * 0.05)(B, S, D)),
            "wqkv": _w((lambda *s: _rng.normal(s) * 0.2)(D, 3 * D)),
            "w_phi": _w((lambda *s: _rng.normal(s) * 0.2)(H, Dh, Dh) * (Dh ** -0.5)),
            "wo": _w((lambda *s: _rng.normal(s) * 0.05)(D, D)),
        }
    _A_in = _A_setup()

    def _B_setup():
        B, S, D, F = 1, 2048, 512, 1792
        return {
            "x": _w((lambda *s: _rng.normal(s) * 0.05)(B, S, D)),
            "w1": _w((lambda *s: _rng.normal(s) * 0.05)(D, F)),
            "b1": _w((lambda *s: _rng.normal(s) * 0.05)(F)),
            "w2": _w((lambda *s: _rng.normal(s) * 0.05)(F, D)),
            "b2": _w((lambda *s: _rng.normal(s) * 0.05)(D)),
        }
    _B_in = _B_setup()

    return {
        "A_x": _A_in["x"],
        "A_wqkv": _A_in["wqkv"],
        "A_w_phi": _A_in["w_phi"],
        "A_wo": _A_in["wo"],
        "B_x": _B_in["x"],
        "B_w1": _B_in["w1"],
        "B_b1": _B_in["b1"],
        "B_w2": _B_in["w2"],
        "B_b2": _B_in["b2"],
    }

def reference(A_x, A_wqkv, A_w_phi, A_wo, B_x, B_w1, B_b1, B_w2, B_b2):
    def _A_ref(x, wqkv, w_phi, wo):
        B, S, D = x.shape
        H = 32; Dh = D // H
        qkv = (lambda x, *d: x.transpose(*d))((x @ wqkv).reshape(B, S, 3, H, Dh), 2, 0, 3, 1, 4)
        q, k, v = qkv[0], qkv[1], qkv[2]
        pq = jnp.einsum("bhsd,hdf->bhsf", q, w_phi)
        pk = jnp.einsum("bhsd,hdf->bhsf", k, w_phi)
        phi_q = jnp.concatenate([_softmax(pq, axis=-1), _softmax(-pq, axis=-1)], axis=-1)
        phi_k = jnp.concatenate([_softmax(pk, axis=-1), _softmax(-pk, axis=-1)], axis=-1)
        kv = jnp.einsum("bhsf,bhsd->bhfd", phi_k, v)
        z  = jnp.einsum("bhsf->bhf", phi_k)
        num = jnp.einsum("bhqf,bhfd->bhqd", phi_q, kv)
        den = jnp.einsum("bhqf,bhf->bhq", phi_q, z)[..., None] + 1e-6
        o = num / den
        return (lambda x, *d: x.transpose(*d))(o, 0, 2, 1, 3).reshape(B, S, D) @ wo

    def _B_ref(x, w1, b1, w2, b2):
        h = jnp.einsum("bsd,df->bsf", x, w1) + b1
        zero = jnp.zeros_like(h)
        r = jnp.where(h > zero, h, zero)
        h = r * r
        out = jnp.einsum("bsf,fd->bsd", h, w2) + b2
        return out

    x = A_x
    h = x + _A_ref(_layernorm(x, axis=-1), A_wqkv, A_w_phi, A_wo)
    h2 = h + _B_ref(_layernorm(h, axis=-1), B_w1, B_b1, B_w2, B_b2)
    return h2
```

```python
import functools
import jax
import jax.numpy as jnp
from jax import lax
import jax.experimental.pallas as pl
import jax.experimental.pallas.tpu as pltpu

F32 = jnp.float32
BF16 = jnp.bfloat16
_NT = (((1,), (1,)), ((), ()))

T_BLK = 512
SUB1 = 1
SUB2 = 2


def _layernorm(xf):
    m = jnp.mean(xf, axis=-1, keepdims=True)
    xc = xf - m
    v = jnp.mean(xc * xc, axis=-1, keepdims=True)
    return xc * lax.rsqrt(v + 1e-5)


def _fold8(a, op):
    return op(a, pltpu.roll(a, 4, 0))


def _hedgehog(p):
    t = p.shape[-1]
    p3 = p.reshape(8, 8, t)
    mx = _fold8(jnp.max(p3, axis=0), jnp.maximum)
    mn = _fold8(jnp.min(p3, axis=0), jnp.minimum)
    ep = jnp.exp(p3 - mx[None])
    en = jnp.exp(mn[None] - p3)
    sp = _fold8(jnp.sum(ep, axis=0), jnp.add)
    sn = _fold8(jnp.sum(en, axis=0), jnp.add)
    pos = ep * (1.0 / sp)[None]
    neg = en * (1.0 / sn)[None]
    return jnp.concatenate([pos.reshape(64, t), neg.reshape(64, t)], axis=0)


def _kernel(x_ref, wqkv_ref, wphi_ref, wo_hbm, w1_hbm, b1_ref, w2_hbm, b2_ref, o_ref,
            wT_ref, phiq_ref, kv_ref, a_ref, wo_ref, w1_ref, w2_ref, sems,
            *, nb, t_blk):
    i = pl.program_id(0)

    def weight_copies():
        return (pltpu.make_async_copy(wo_hbm, wo_ref, sems.at[0]),
                pltpu.make_async_copy(w1_hbm, w1_ref, sems.at[1]),
                pltpu.make_async_copy(w2_hbm, w2_ref, sems.at[2]))

    @pl.when(i == 0)
    def _init():
        for c in weight_copies():
            c.start()
        w2d = wphi_ref[...].reshape(256, 32)
        r32 = lax.broadcasted_iota(jnp.int32, (512, 32), 0)
        c32 = lax.broadcasted_iota(jnp.int32, (512, 32), 1)
        selh = jnp.where(((r32 // 64) * 4 + r32 % 4) == c32, 1.0, 0.0).astype(BF16)
        r1 = lax.dot_general(selh, w2d, _NT, preferred_element_type=F32)
        rr = lax.broadcasted_iota(jnp.int32, (512, 256), 0)
        cc = lax.broadcasted_iota(jnp.int32, (512, 256), 1)
        r2 = jnp.where(((rr % 64) // 4) == (cc % 16), r1, 0.0).astype(BF16)
        kc = lax.broadcasted_iota(jnp.int32, (256, 128), 0)
        nc = lax.broadcasted_iota(jnp.int32, (256, 128), 1)
        coll = jnp.where((kc // 16) == (nc % 16), 1.0, 0.0).astype(BF16)
        r3 = jnp.dot(r2, coll, preferred_element_type=F32)
        r = lax.broadcasted_iota(jnp.int32, (512, 128), 0)
        c = lax.broadcasted_iota(jnp.int32, (512, 128), 1)
        same_head = (((r % 128) // 64) * 4 + r % 4) == (c // 16)
        bd_all = jnp.where(same_head, r3, 0.0).astype(BF16)
        re = lax.broadcasted_iota(jnp.int32, (128, 128), 0)
        ce = lax.broadcasted_iota(jnp.int32, (128, 128), 1)
        eye = jnp.where(re == ce, 1.0, 0.0).astype(BF16)
        for g in range(4):
            bd = bd_all[g * 128:(g + 1) * 128, :]
            for s in range(3):
                w = wqkv_ref[:, s * 512 + g * 128: s * 512 + (g + 1) * 128]
                lhs = bd if s < 2 else eye
                wt = lax.dot_general(lhs, w, _NT, preferred_element_type=F32)
                wT_ref[s * 512 + g * 128: s * 512 + (g + 1) * 128, :] = wt.astype(BF16)
        kv_ref[...] = jnp.zeros(kv_ref.shape, F32)

    @pl.when(i < nb)
    def _phase1():
        ts = t_blk // SUB1
        ones = jnp.ones((16, ts), BF16)
        for sb in range(SUB1):
            xf = x_ref[sb * ts:(sb + 1) * ts, :].astype(F32)
            xn = _layernorm(xf).astype(BF16)
            pT = lax.dot_general(wT_ref[...], xn, _NT, preferred_element_type=F32)
            for j in range(8):
                phiq_ref[i, j * 128:(j + 1) * 128, sb * ts:(sb + 1) * ts] = _hedgehog(
                    pT[j * 64:(j + 1) * 64, :]).astype(BF16)
            for j in range(8):
                pk = _hedgehog(pT[512 + j * 64: 512 + (j + 1) * 64, :]).astype(BF16)
                vt = pT[1024 + j * 64: 1024 + (j + 1) * 64, :].astype(BF16)
                lhs = jnp.concatenate([vt, ones], axis=0)
                kv_ref[j] += lax.dot_general(lhs, pk, _NT, preferred_element_type=F32)

    @pl.when(i == nb)
    def _finalize():
        r = lax.broadcasted_iota(jnp.int32, (80, 128), 0)
        c = lax.broadcasted_iota(jnp.int32, (80, 128), 1)
        head = jnp.where(r < 64, r // 16, r - 64)
        keep = head == (c % 4)
        for j in range(8):
            a_ref[j] = jnp.where(keep, kv_ref[j], 0.0).astype(BF16)
        for cpy in weight_copies():
            cpy.wait()

    @pl.when(i >= nb)
    def _phase2():
        jb = i - nb
        ts = t_blk // SUB2
        b1 = b1_ref[...].astype(F32).reshape(1, -1)
        b2 = b2_ref[...].astype(F32).reshape(1, -1)
        sls = [slice(sb * ts, (sb + 1) * ts) for sb in range(SUB2)]
        os_ = []
        for sb in range(SUB2):
            outs = []
            for j in range(8):
                nd = jnp.dot(a_ref[j], phiq_ref[jb, j * 128:(j + 1) * 128, sls[sb]],
                             preferred_element_type=F32)
                inv = 1.0 / (nd[64:72, :] + 1e-6)
                for hh in range(4):
                    outs.append(nd[hh * 16:(hh + 1) * 16, :]
                                * jnp.broadcast_to(inv[hh:hh + 1, :], (16, ts)))
            oT = jnp.concatenate(outs, axis=0)
            os_.append(oT.T.astype(BF16))
        hs, hns = [], []
        for sb in range(SUB2):
            h = (x_ref[sls[sb], :].astype(F32)
                 + jnp.dot(os_[sb], wo_ref[...], preferred_element_type=F32))
            hs.append(h)
            hns.append(_layernorm(h).astype(BF16))
        for sb in range(SUB2):
            h1 = jnp.dot(hns[sb], w1_ref[...], preferred_element_type=F32) + b1
            r1 = jnp.maximum(h1, 0.0)
            act = (r1 * r1).astype(BF16)
            y = jnp.dot(act, w2_ref[...], preferred_element_type=F32) + b2
            o_ref[sls[sb], :] = (hs[sb] + y).astype(o_ref.dtype)


@jax.jit
def pallas_sequential_preLN__linear_kernel_hedgehog__dense_activation_squared_relu__prompt_kernel(
    A_x: jax.Array,
    A_wqkv: jax.Array,
    A_w_phi: jax.Array,
    A_wo: jax.Array,
    B_x: jax.Array,
    B_w1: jax.Array,
    B_b1: jax.Array,
    B_w2: jax.Array,
    B_b2: jax.Array,
):
    B, S, D = A_x.shape
    H, Dh, _ = A_w_phi.shape
    F = B_w1.shape[1]
    assert (B, D, H, Dh) == (1, 512, 32, 16)
    t_blk = T_BLK
    nb = S // t_blk

    x2 = A_x.reshape(S, D)

    const = lambda i: (0, 0)
    out = pl.pallas_call(
        functools.partial(_kernel, nb=nb, t_blk=t_blk),
        grid=(2 * nb,),
        in_specs=[
            pl.BlockSpec((t_blk, D), lambda i: (i % nb, 0)),
            pl.BlockSpec((D, 3 * D), const),
            pl.BlockSpec((Dh, Dh, H), lambda i: (0, 0, 0)),
            pl.BlockSpec(memory_space=pl.ANY),
            pl.BlockSpec(memory_space=pl.ANY),
            pl.BlockSpec((F,), lambda i: (0,)),
            pl.BlockSpec(memory_space=pl.ANY),
            pl.BlockSpec((D,), lambda i: (0,)),
        ],
        out_specs=pl.BlockSpec((t_blk, D), lambda i: (jnp.maximum(i - nb, 0), 0)),
        out_shape=jax.ShapeDtypeStruct((S, D), A_x.dtype),
        scratch_shapes=[
            pltpu.VMEM((3 * D, D), BF16),
            pltpu.VMEM((nb, 2 * D, t_blk), BF16),
            pltpu.VMEM((8, 80, 128), F32),
            pltpu.VMEM((8, 80, 128), BF16),
            pltpu.VMEM((D, D), BF16),
            pltpu.VMEM((D, F), BF16),
            pltpu.VMEM((F, D), BF16),
            pltpu.SemaphoreType.DMA((3,)),
        ],
        compiler_params=pltpu.CompilerParams(
            dimension_semantics=("arbitrary",),
            vmem_limit_bytes=100 * 1024 * 1024,
        ),
    )(x2, A_wqkv, jnp.transpose(A_w_phi, (1, 2, 0)), A_wo, B_w1, B_b1, B_w2, B_b2)
    return out.reshape(B, S, D)
```

```python
import functools
import jax
import jax.numpy as jnp
from jax import lax
import jax.experimental.pallas as pl
import jax.experimental.pallas.tpu as pltpu

F32 = jnp.float32
BF16 = jnp.bfloat16
_NT = (((1,), (1,)), ((), ()))

LOG2E = 1.4426950408889634
T_BLK = 512
SUB2 = 2
UNROLL1 = True
UNROLL2 = False


def _layernorm(xf):
    m = jnp.mean(xf, axis=-1, keepdims=True)
    xc = xf - m
    v = jnp.mean(xc * xc, axis=-1, keepdims=True)
    return xc * lax.rsqrt(v + 1e-5)


def _fold8(a, op):
    return op(a, pltpu.roll(a, 4, 0))


def _hedgehog(p):
    t = p.shape[-1]
    p3 = p.reshape(8, 8, t)
    mx = _fold8(jnp.max(p3, axis=0), jnp.maximum)
    mn = _fold8(jnp.min(p3, axis=0), jnp.minimum)
    ep = jnp.exp2(p3 - mx[None])
    en = jnp.exp2(mn[None] - p3)
    sp = _fold8(jnp.sum(ep, axis=0), jnp.add)
    sn = _fold8(jnp.sum(en, axis=0), jnp.add)
    pos = ep * (1.0 / sp)[None]
    neg = en * (1.0 / sn)[None]
    return jnp.concatenate([pos.reshape(64, t), neg.reshape(64, t)], axis=0)


def _kernel(x_hbm, wqkv_hbm, wphi_hbm, wo_hbm, w1_hbm, b1_hbm, w2_hbm, b2_hbm, out_hbm,
            wphi_ref, b1_ref, b2_ref, x_ref, wqkv_ref, wqT_ref, wkT_ref, wvT_ref, phiq_ref, kv_ref, a_ref, wo_ref, w1_ref, w2_ref,
            obuf_ref, xsem, wsem, osem, *, nb, t_blk):
    T = t_blk
    D = 512

    TH = T // 2
    wT_refs = (wqT_ref, wkT_ref, wvT_ref)

    def x_copy(b):
        return pltpu.make_async_copy(x_hbm.at[pl.ds(b * T, T), :], x_ref.at[pl.ds(b * T, T), :],
                                     xsem.at[b])

    def x0_copy(half):
        return pltpu.make_async_copy(x_hbm.at[pl.ds(half * TH, TH), :],
                                     x_ref.at[pl.ds(half * TH, TH), :], xsem.at[half * nb])

    def wqkv_copy(s):
        return pltpu.make_async_copy(wqkv_hbm.at[:, pl.ds(s * D, D)],
                                     wqkv_ref.at[:, pl.ds(s * D, D)], wsem.at[s])

    late_copies = (pltpu.make_async_copy(wo_hbm, wo_ref, wsem.at[3]),
                   pltpu.make_async_copy(w1_hbm, w1_ref, wsem.at[4]),
                   pltpu.make_async_copy(w2_hbm, w2_ref, wsem.at[5]),
                   pltpu.make_async_copy(b1_hbm, b1_ref, wsem.at[6]),
                   pltpu.make_async_copy(b2_hbm, b2_ref, wsem.at[7]))
    wphi_copy = pltpu.make_async_copy(wphi_hbm, wphi_ref, wsem.at[8])

    wphi_copy.start()
    x0_copy(0).start()
    wqkv_copy(0).start()
    x0_copy(1).start()
    wphi_copy.wait()

    w2d = wphi_ref[...].reshape(256, 32)
    r32 = lax.broadcasted_iota(jnp.int32, (512, 32), 0)
    c32 = lax.broadcasted_iota(jnp.int32, (512, 32), 1)
    selh = jnp.where(((r32 // 64) * 4 + r32 % 4) == c32, 1.0, 0.0).astype(BF16)
    r1 = lax.dot_general(selh, w2d, _NT, preferred_element_type=F32)
    rr = lax.broadcasted_iota(jnp.int32, (512, 256), 0)
    cc = lax.broadcasted_iota(jnp.int32, (512, 256), 1)
    r2 = jnp.where(((rr % 64) // 4) == (cc % 16), r1, 0.0).astype(BF16)
    kc = lax.broadcasted_iota(jnp.int32, (256, 128), 0)
    nc = lax.broadcasted_iota(jnp.int32, (256, 128), 1)
    coll = jnp.where((kc // 16) == (nc % 16), 1.0, 0.0).astype(BF16)
    r3 = jnp.dot(r2, coll, preferred_element_type=F32)
    r = lax.broadcasted_iota(jnp.int32, (512, 128), 0)
    c = lax.broadcasted_iota(jnp.int32, (512, 128), 1)
    same_head = (((r % 128) // 64) * 4 + r % 4) == (c // 16)
    bd_all = jnp.where(same_head, r3, 0.0).astype(BF16)

    def fold(s):
        for g in range(4):
            w = wqkv_ref[:, s * D + g * 128: s * D + (g + 1) * 128]
            wt = lax.dot_general(bd_all[g * 128:(g + 1) * 128, :], w, _NT,
                                 preferred_element_type=F32)
            wT_refs[s][g * 128:(g + 1) * 128, :] = (wt * LOG2E).astype(BF16)

    def transpose_v():
        for g in range(4):
            w = wqkv_ref[:, 2 * D + g * 128: 2 * D + (g + 1) * 128].astype(F32)
            wvT_ref[g * 128:(g + 1) * 128, :] = w.T.astype(BF16)

    def ln1(row0, n=T):
        return _layernorm(x_ref[pl.ds(row0, n), :].astype(F32)).astype(BF16)

    def proj(s, xn):
        return lax.dot_general(wT_refs[s][...], xn, _NT,
                               preferred_element_type=F32)

    def q_part(b, pq, col=0):
        n = pq.shape[1]
        for j in range(8):
            phiq_ref[b, j * 128:(j + 1) * 128, col:col + n] = _hedgehog(
                pq[j * 64:(j + 1) * 64, :]).astype(BF16)

    ones = jnp.ones((16, T), BF16)

    def k_part(pk):
        return [_hedgehog(pk[j * 64:(j + 1) * 64, :]).astype(BF16) for j in range(8)]

    def kv_part(fks, vt, first):
        for j in range(8):
            lhs = jnp.concatenate([vt[j * 64:(j + 1) * 64, :].astype(BF16), ones], axis=0)
            upd = lax.dot_general(lhs, fks[j], _NT, preferred_element_type=F32)
            if first:
                kv_ref[j] = upd
            else:
                kv_ref[j] += upd

    x0_copy(0).wait()
    xa = ln1(0, TH)
    wqkv_copy(0).wait()
    wqkv_copy(1).start()
    fold(0)
    x0_copy(1).wait()
    x_copy(1).start()
    wqkv_copy(2).start()
    pqa = proj(0, xa)
    xb = ln1(TH, TH)
    pqb = proj(0, xb)
    q_part(0, pqa, 0)
    q_part(0, pqb, TH)
    xn0 = jnp.concatenate([xa, xb], axis=0)
    wqkv_copy(1).wait()
    x_copy(1).wait()
    for b in range(2, nb):
        x_copy(b).start()
    fold(1)
    pk = proj(1, xn0)
    fks0 = k_part(pk)
    xn1 = ln1(T)
    pq = proj(0, xn1)
    q_part(1, pq)
    wqkv_copy(2).wait()
    for b in range(2, nb):
        x_copy(b).wait()
    for cp in late_copies:
        cp.start()
    transpose_v()
    pk = proj(1, xn1)
    vt = proj(2, xn0)
    kv_part(fks0, vt, True)
    vt = proj(2, xn1)
    xn = ln1(2 * T)
    kv_part(k_part(pk), vt, False)

    for b in range(2, nb):
        pq = proj(0, xn)
        pk = proj(1, xn)
        vt = proj(2, xn)
        if b + 1 < nb:
            xn = ln1((b + 1) * T)
        q_part(b, pq)
        kv_part(k_part(pk), vt, False)

    r = lax.broadcasted_iota(jnp.int32, (80, 128), 0)
    c = lax.broadcasted_iota(jnp.int32, (80, 128), 1)
    head = jnp.where(r < 64, r // 16, r - 64)
    keep = head == (c % 4)
    for j in range(8):
        a_ref[j] = jnp.where(keep, kv_ref[j], 0.0).astype(BF16)
    for cp in late_copies:
        cp.wait()

    ts = T // SUB2
    b1 = b1_ref[...].astype(F32).reshape(1, -1)
    b2 = b2_ref[...].astype(F32).reshape(1, -1)

    def out_copy(row0, n, k):
        return pltpu.make_async_copy(obuf_ref.at[pl.ds(row0, n), :],
                                     out_hbm.at[pl.ds(row0, n), :], osem.at[k])

    def p2_body(b, carry):
        rows = [b * T + sb * ts for sb in range(SUB2)]
        if not isinstance(b, int):
            rows = [pl.multiple_of(r0, ts) for r0 in rows]
        sls = [slice(sb * ts, (sb + 1) * ts) for sb in range(SUB2)]
        os_ = []
        for sb in range(SUB2):
            outs = []
            for j in range(8):
                nd = jnp.dot(a_ref[j], phiq_ref[b, j * 128:(j + 1) * 128, sls[sb]],
                             preferred_element_type=F32)
                inv = 1.0 / (nd[64:72, :] + 1e-6)
                for hh in range(4):
                    outs.append(nd[hh * 16:(hh + 1) * 16, :]
                                * jnp.broadcast_to(inv[hh:hh + 1, :], (16, ts)))
            oT = jnp.concatenate(outs, axis=0)
            os_.append(oT.T.astype(BF16))
        hs, hns = [], []
        for sb in range(SUB2):
            h = (x_ref[pl.ds(rows[sb], ts), :].astype(F32)
                 + jnp.dot(os_[sb], wo_ref[...], preferred_element_type=F32))
            hs.append(h)
            hns.append(_layernorm(h).astype(BF16))
        for sb in range(SUB2):
            h1 = jnp.dot(hns[sb], w1_ref[...], preferred_element_type=F32) + b1
            r1 = jnp.maximum(h1, 0.0)
            act = (r1 * r1).astype(BF16)
            if sb < SUB2 - 1:
                y = jnp.dot(act, w2_ref[...], preferred_element_type=F32) + b2
                obuf_ref[pl.ds(rows[sb], ts), :] = (hs[sb] + y).astype(obuf_ref.dtype)
                out_copy(rows[sb], ts, b * (SUB2 + 1) + sb).start()
            else:
                th = ts // 2
                for hf in range(2):
                    y = jnp.dot(act[hf * th:(hf + 1) * th], w2_ref[...], preferred_element_type=F32) + b2
                    r0 = rows[sb] + hf * th
                    obuf_ref[pl.ds(r0, th), :] = (hs[sb][hf * th:(hf + 1) * th] + y).astype(obuf_ref.dtype)
                    out_copy(r0, th, b * (SUB2 + 1) + sb + hf).start()
        return carry

    if UNROLL2:
        for b in range(nb):
            p2_body(b, 0)
    else:
        def p2_body2(bb, carry):
            p2_body(2 * bb, carry)
            p2_body(2 * bb + 1, carry)
            return carry
        lax.fori_loop(0, nb // 2, p2_body2, 0)
    for b in range(nb):
        for sb in range(SUB2 - 1):
            out_copy(b * T + sb * ts, ts, b * (SUB2 + 1) + sb).wait()
        for hf in range(2):
            out_copy(b * T + (SUB2 - 1) * ts + hf * (ts // 2), ts // 2, b * (SUB2 + 1) + SUB2 - 1 + hf).wait()


@jax.jit
def pallas_sequential_preLN__linear_kernel_hedgehog__dense_activation_squared_relu__prompt_kernel(
    A_x: jax.Array,
    A_wqkv: jax.Array,
    A_w_phi: jax.Array,
    A_wo: jax.Array,
    B_x: jax.Array,
    B_w1: jax.Array,
    B_b1: jax.Array,
    B_w2: jax.Array,
    B_b2: jax.Array,
):
    B, S, D = A_x.shape
    H, Dh, _ = A_w_phi.shape
    F = B_w1.shape[1]
    assert (B, D, H, Dh) == (1, 512, 32, 16)
    t_blk = T_BLK
    nb = S // t_blk

    x2 = A_x.reshape(S, D)
    vmem = pl.BlockSpec(memory_space=pltpu.VMEM)
    hbm = pl.BlockSpec(memory_space=pl.ANY)
    out = pl.pallas_call(
        functools.partial(_kernel, nb=nb, t_blk=t_blk),
        in_specs=[hbm] * 8,
        out_specs=hbm,
        out_shape=jax.ShapeDtypeStruct((S, D), A_x.dtype),
        scratch_shapes=[
            pltpu.VMEM((Dh, Dh, H), BF16),
            pltpu.VMEM((F,), BF16),
            pltpu.VMEM((D,), BF16),
            pltpu.VMEM((S, D), BF16),
            pltpu.VMEM((D, 3 * D), BF16),
            pltpu.VMEM((D, D), BF16),
            pltpu.VMEM((D, D), BF16),
            pltpu.VMEM((D, D), BF16),
            pltpu.VMEM((nb, 2 * D, t_blk), BF16),
            pltpu.VMEM((8, 80, 128), F32),
            pltpu.VMEM((8, 80, 128), BF16),
            pltpu.VMEM((D, D), BF16),
            pltpu.VMEM((D, F), BF16),
            pltpu.VMEM((F, D), BF16),
            pltpu.VMEM((S, D), BF16),
            pltpu.SemaphoreType.DMA((nb + 1,)),
            pltpu.SemaphoreType.DMA((9,)),
            pltpu.SemaphoreType.DMA((nb * (SUB2 + 1),)),
        ],
        compiler_params=pltpu.CompilerParams(
            vmem_limit_bytes=100 * 1024 * 1024,
        ),
    )(x2, A_wqkv, jnp.transpose(A_w_phi, (1, 2, 0)), A_wo, B_w1, B_b1, B_w2, B_b2)
    return out.reshape(B, S, D)
```

```python
import functools
import jax
import jax.numpy as jnp
from jax import lax
import jax.experimental.pallas as pl
import jax.experimental.pallas.tpu as pltpu

F32 = jnp.float32
BF16 = jnp.bfloat16
_NT = (((1,), (1,)), ((), ()))

LOG2E = 1.4426950408889634
T_BLK = 512
SUB2 = 2


def _layernorm(xf):
    m = jnp.mean(xf, axis=-1, keepdims=True)
    xc = xf - m
    v = jnp.mean(xc * xc, axis=-1, keepdims=True)
    return xc * lax.rsqrt(v + 1e-5)


def _fold8(a, op):
    return op(a, pltpu.roll(a, 4, 0))


def _hedgehog(p):
    t = p.shape[-1]
    p3 = p.reshape(8, 8, t)
    mx = _fold8(jnp.max(p3, axis=0), jnp.maximum)
    mn = _fold8(jnp.min(p3, axis=0), jnp.minimum)
    ep = jnp.exp2(p3 - mx[None])
    en = jnp.exp2(mn[None] - p3)
    sp = _fold8(jnp.sum(ep, axis=0), jnp.add)
    sn = _fold8(jnp.sum(en, axis=0), jnp.add)
    pos = ep * (1.0 / sp)[None]
    neg = en * (1.0 / sn)[None]
    return jnp.concatenate([pos.reshape(64, t), neg.reshape(64, t)], axis=0)


def _kernel(x_hbm, wqkv_hbm, wphi_hbm, wo_hbm, w1_hbm, b1_hbm, w2_hbm, b2_hbm, out_hbm,
            wphi_ref, b1_ref, b2_ref, x_ref, wqkv_ref, wqT_ref, wkT_ref, wvT_ref, phiq_ref,
            kv_ref, a_ref, wo_ref, w1_ref, w2_ref, obuf_ref, xsem, wsem, osem, *, nb, t_blk):
    T = t_blk
    D = 512
    TA = 128
    wT_refs = (wqT_ref, wkT_ref, wvT_ref)

    def x_copy(b):
        return pltpu.make_async_copy(x_hbm.at[pl.ds(b * T, T), :], x_ref.at[pl.ds(b * T, T), :],
                                     xsem.at[b])

    def x0_copy(half):
        r0, n = (0, TA) if half == 0 else (TA, T - TA)
        return pltpu.make_async_copy(x_hbm.at[pl.ds(r0, n), :],
                                     x_ref.at[pl.ds(r0, n), :], xsem.at[half * nb])

    def wqkv_copy(s):
        return pltpu.make_async_copy(wqkv_hbm.at[:, pl.ds(s * D, D)],
                                     wqkv_ref.at[:, pl.ds(s * D, D)], wsem.at[s])

    late_copies = (pltpu.make_async_copy(wo_hbm, wo_ref, wsem.at[3]),
                   pltpu.make_async_copy(w1_hbm, w1_ref, wsem.at[4]),
                   pltpu.make_async_copy(w2_hbm, w2_ref, wsem.at[5]),
                   pltpu.make_async_copy(b1_hbm, b1_ref, wsem.at[6]),
                   pltpu.make_async_copy(b2_hbm, b2_ref, wsem.at[7]))
    wphi_copy = pltpu.make_async_copy(wphi_hbm, wphi_ref, wsem.at[8])

    wphi_copy.start()
    x0_copy(0).start()
    wqkv_copy(2).start()

    def make_bd():
        w2d = wphi_ref[...].reshape(256, 32)
        r32 = lax.broadcasted_iota(jnp.int32, (512, 32), 0)
        c32 = lax.broadcasted_iota(jnp.int32, (512, 32), 1)
        selh = jnp.where(((r32 // 64) * 4 + r32 % 4) == c32, 1.0, 0.0).astype(BF16)
        r1 = lax.dot_general(selh, w2d, _NT, preferred_element_type=F32)
        rr = lax.broadcasted_iota(jnp.int32, (512, 256), 0)
        cc = lax.broadcasted_iota(jnp.int32, (512, 256), 1)
        r2 = jnp.where(((rr % 64) // 4) == (cc % 16), r1, 0.0).astype(BF16)
        kc = lax.broadcasted_iota(jnp.int32, (256, 128), 0)
        nc = lax.broadcasted_iota(jnp.int32, (256, 128), 1)
        coll = jnp.where((kc // 16) == (nc % 16), 1.0, 0.0).astype(BF16)
        r3 = jnp.dot(r2, coll, preferred_element_type=F32)
        r = lax.broadcasted_iota(jnp.int32, (512, 128), 0)
        c = lax.broadcasted_iota(jnp.int32, (512, 128), 1)
        same_head = (((r % 128) // 64) * 4 + r % 4) == (c // 16)
        bd_all = jnp.where(same_head, r3, 0.0).astype(BF16)
        return bd_all

    def fold(s, bd_all):
        for g in range(4):
            w = wqkv_ref[:, s * D + g * 128: s * D + (g + 1) * 128]
            wt = lax.dot_general(bd_all[g * 128:(g + 1) * 128, :], w, _NT,
                                 preferred_element_type=F32)
            wT_refs[s][g * 128:(g + 1) * 128, :] = (wt * LOG2E).astype(BF16)

    def transpose_v():
        for g in range(4):
            w = wqkv_ref[:, 2 * D + g * 128: 2 * D + (g + 1) * 128].astype(F32)
            wvT_ref[g * 128:(g + 1) * 128, :] = w.T.astype(BF16)

    def ln1(row0, n=T):
        return _layernorm(x_ref[pl.ds(row0, n), :].astype(F32)).astype(BF16)

    def proj(s, xn):
        return lax.dot_general(wT_refs[s][...], xn, _NT,
                               preferred_element_type=F32)

    def q_part(b, pq, col=0):
        n = pq.shape[1]
        for j in range(8):
            phiq_ref[b, j * 128:(j + 1) * 128, col:col + n] = _hedgehog(
                pq[j * 64:(j + 1) * 64, :]).astype(BF16)

    ones = jnp.ones((16, T), BF16)

    def k_part(pk):
        return [_hedgehog(pk[j * 64:(j + 1) * 64, :]).astype(BF16) for j in range(8)]

    def kv_part(fks, vt, first):
        for j in range(8):
            lhs = jnp.concatenate([vt[j * 64:(j + 1) * 64, :].astype(BF16), ones], axis=0)
            upd = lax.dot_general(lhs, fks[j], _NT, preferred_element_type=F32)
            if first:
                kv_ref[j] = upd
            else:
                kv_ref[j] += upd

    wphi_copy.wait()
    bd_all = make_bd()
    x0_copy(0).wait()
    x0_copy(1).start()
    xa = ln1(0, TA)
    wqkv_copy(2).wait()
    wqkv_copy(1).start()
    transpose_v()
    x0_copy(1).wait()
    x_copy(1).start()
    vta = proj(2, xa)
    xb = ln1(TA, T - TA)
    vtb = proj(2, xb)
    xn0 = jnp.concatenate([xa, xb], axis=0)
    vt0 = jnp.concatenate([vta, vtb], axis=1).astype(BF16)
    wqkv_copy(1).wait()
    x_copy(1).wait()
    wqkv_copy(0).start()
    for b in range(2, nb):
        x_copy(b).start()
    fold(1, bd_all)
    pk = proj(1, xn0)
    fks0 = k_part(pk)
    xn1 = ln1(T)
    vt1 = proj(2, xn1)
    kv_part(fks0, vt0, True)
    wqkv_copy(0).wait()
    for b in range(2, nb):
        x_copy(b).wait()
    for cp in late_copies:
        cp.start()
    fold(0, bd_all)
    pk = proj(1, xn1)
    pq = proj(0, xn0)
    fks = k_part(pk)
    q_part(0, pq)
    kv_part(fks, vt1, False)
    pq = proj(0, xn1)
    xn = ln1(2 * T)
    q_part(1, pq)

    for b in range(2, nb):
        vt = proj(2, xn)
        pk = proj(1, xn)
        pq = proj(0, xn)
        if b + 1 < nb:
            xn = ln1((b + 1) * T)
        fks = k_part(pk)
        q_part(b, pq)
        kv_part(fks, vt, False)

    r = lax.broadcasted_iota(jnp.int32, (80, 128), 0)
    c = lax.broadcasted_iota(jnp.int32, (80, 128), 1)
    head = jnp.where(r < 64, r // 16, r - 64)
    keep = head == (c % 4)
    for j in range(8):
        a_ref[j] = jnp.where(keep, kv_ref[j], 0.0).astype(BF16)
    for cp in late_copies:
        cp.wait()

    ts = T // SUB2
    b1 = b1_ref[...].astype(F32).reshape(1, -1)
    b2 = b2_ref[...].astype(F32).reshape(1, -1)

    def out_copy(row0, n, k):
        return pltpu.make_async_copy(obuf_ref.at[pl.ds(row0, n), :],
                                     out_hbm.at[pl.ds(row0, n), :], osem.at[k])

    def p2_block(b):
        rows = [pl.multiple_of(b * T + sb * ts, ts) for sb in range(SUB2)]
        sls = [slice(sb * ts, (sb + 1) * ts) for sb in range(SUB2)]
        os_ = []
        for sb in range(SUB2):
            outs = []
            for j in range(8):
                nd = jnp.dot(a_ref[j], phiq_ref[b, j * 128:(j + 1) * 128, sls[sb]],
                             preferred_element_type=F32)
                inv = 1.0 / (nd[64:72, :] + 1e-6)
                for hh in range(4):
                    outs.append(nd[hh * 16:(hh + 1) * 16, :]
                                * jnp.broadcast_to(inv[hh:hh + 1, :], (16, ts)))
            oT = jnp.concatenate(outs, axis=0)
            os_.append(oT.T.astype(BF16))
        hs, hns = [], []
        for sb in range(SUB2):
            h = (x_ref[pl.ds(rows[sb], ts), :].astype(F32)
                 + jnp.dot(os_[sb], wo_ref[...], preferred_element_type=F32))
            hs.append(h)
            hns.append(_layernorm(h).astype(BF16))
        for sb in range(SUB2):
            h1 = jnp.dot(hns[sb], w1_ref[...], preferred_element_type=F32) + b1
            r1 = jnp.maximum(h1, 0.0)
            act = (r1 * r1).astype(BF16)
            if sb < SUB2 - 1:
                y = jnp.dot(act, w2_ref[...], preferred_element_type=F32) + b2
                obuf_ref[pl.ds(rows[sb], ts), :] = (hs[sb] + y).astype(obuf_ref.dtype)
                out_copy(rows[sb], ts, b * (SUB2 + 1) + sb).start()
            else:
                th = ts // 2
                for hf in range(2):
                    y = jnp.dot(act[hf * th:(hf + 1) * th], w2_ref[...],
                                preferred_element_type=F32) + b2
                    r0 = rows[sb] + hf * th
                    obuf_ref[pl.ds(r0, th), :] = (
                        hs[sb][hf * th:(hf + 1) * th] + y).astype(obuf_ref.dtype)
                    out_copy(r0, th, b * (SUB2 + 1) + sb + hf).start()

    def p2_body(bb, carry):
        p2_block(2 * bb)
        p2_block(2 * bb + 1)
        return carry

    lax.fori_loop(0, nb // 2, p2_body, 0)
    for b in range(nb):
        for sb in range(SUB2 - 1):
            out_copy(b * T + sb * ts, ts, b * (SUB2 + 1) + sb).wait()
        for hf in range(2):
            out_copy(b * T + (SUB2 - 1) * ts + hf * (ts // 2), ts // 2,
                     b * (SUB2 + 1) + SUB2 - 1 + hf).wait()


@jax.jit
def pallas_sequential_preLN__linear_kernel_hedgehog__dense_activation_squared_relu__prompt_kernel(
    A_x: jax.Array,
    A_wqkv: jax.Array,
    A_w_phi: jax.Array,
    A_wo: jax.Array,
    B_x: jax.Array,
    B_w1: jax.Array,
    B_b1: jax.Array,
    B_w2: jax.Array,
    B_b2: jax.Array,
):
    B, S, D = A_x.shape
    H, Dh, _ = A_w_phi.shape
    F = B_w1.shape[1]
    t_blk = T_BLK
    nb = S // t_blk
    assert (B, D, H, Dh) == (1, 512, 32, 16) and S % (2 * t_blk) == 0 and nb >= 4

    x2 = A_x.reshape(S, D)
    hbm = pl.BlockSpec(memory_space=pl.ANY)
    out = pl.pallas_call(
        functools.partial(_kernel, nb=nb, t_blk=t_blk),
        in_specs=[hbm] * 8,
        out_specs=hbm,
        out_shape=jax.ShapeDtypeStruct((S, D), A_x.dtype),
        scratch_shapes=[
            pltpu.VMEM((Dh, Dh, H), BF16),
            pltpu.VMEM((F,), BF16),
            pltpu.VMEM((D,), BF16),
            pltpu.VMEM((S, D), BF16),
            pltpu.VMEM((D, 3 * D), BF16),
            pltpu.VMEM((D, D), BF16),
            pltpu.VMEM((D, D), BF16),
            pltpu.VMEM((D, D), BF16),
            pltpu.VMEM((nb, 2 * D, t_blk), BF16),
            pltpu.VMEM((8, 80, 128), F32),
            pltpu.VMEM((8, 80, 128), BF16),
            pltpu.VMEM((D, D), BF16),
            pltpu.VMEM((D, F), BF16),
            pltpu.VMEM((F, D), BF16),
            pltpu.VMEM((S, D), BF16),
            pltpu.SemaphoreType.DMA((nb + 1,)),
            pltpu.SemaphoreType.DMA((9,)),
            pltpu.SemaphoreType.DMA((nb * (SUB2 + 1),)),
        ],
        compiler_params=pltpu.CompilerParams(
            vmem_limit_bytes=100 * 1024 * 1024,
        ),
    )(x2, A_wqkv, jnp.transpose(A_w_phi, (1, 2, 0)), A_wo, B_w1, B_b1, B_w2, B_b2)
    return out.reshape(B, S, D)
```
